```python
import jax
import jax.numpy as jnp

def _softmax(x, axis=-1):
    return jax.nn.softmax(x, axis=axis)
def _gelu(x):
    return jax.nn.gelu(x, approximate=True)
def _silu(x):
    return jax.nn.silu(x)
def _sigmoid(x):
    return jax.nn.sigmoid(x)
def _layernorm(x, axis=-1, eps=1e-5):
    m = jnp.mean(x, axis=axis, keepdims=True)
    v = jnp.var(x, axis=axis, keepdims=True)
    return (x - m) / jnp.sqrt(v + eps)
def _scatter_add(tgt, idx, src, axis=0):
    return tgt.at[idx].add(src)
def _segment_sum(src, seg, n):
    return jax.ops.segment_sum(src, seg, n)
class _Rng:
    def __init__(self, key):
        self._k = key
    def _next(self):
        self._k, sub = jax.random.split(self._k)
        return sub
    def normal(self, shape):
        return jax.random.normal(self._next(), shape, dtype=jnp.bfloat16)
    def randint(self, lo, hi, shape):
        return jax.random.randint(self._next(), shape, lo, hi, dtype=jnp.int32)
    def uniform(self, shape, lo=0.0, hi=1.0):
        return jax.random.uniform(self._next(), shape, jnp.bfloat16, lo, hi)
    def permutation(self, n):
        return jax.random.permutation(self._next(), n)


kernel_name = 'recurrent_scan__sliding_block_cached__mixer_s_mlp__decode'

def _fwd_setup_inputs():
    _rng = _Rng(jax.random.key(int.from_bytes(__import__("os").urandom(4), "little")))
    _w = (lambda a: (lambda t: t.astype(jnp.bfloat16) if jnp.issubdtype(t.dtype, jnp.floating) else t)(jnp.asarray(a)))
    def _A_setup():
        B, Sq, D = 4, 1, 512
        Hq, Hkv, Sk, Dh = 32, 8, 8192, 128
        assert Hq % Hkv == 0, (Hq, Hkv)
        return {
            "x": _w((lambda *s: _rng.normal(s) * 0.05)(B, Sq, D)),
            "k_cache": _w((lambda *s: _rng.normal(s) * 0.05)(B, Hkv, Sk, Dh)),
            "v_cache": _w((lambda *s: _rng.normal(s) * 0.05)(B, Hkv, Sk, Dh)),
            "wq": _w((lambda *s: _rng.normal(s) * 0.05)(D, Hq * Dh) * (D ** -0.5)),
            "wo": _w((lambda *s: _rng.normal(s) * 0.05)(Hq * Dh, D) * ((Hq * Dh) ** -0.5)),
        }
    _A_in = _A_setup()

    def _B_setup():
        B, S, D, F = 4, 1, 512, 1792
        return {
            "x":  _w((lambda *s: _rng.normal(s) * 0.05)(B, S, D)),
            "w1": _w((lambda *s: _rng.normal(s) * 0.05)(D, D) * (D ** -0.5)),
            "w2": _w((lambda *s: _rng.normal(s) * 0.05)(D, D) * (D ** -0.5)),
            "w3": _w((lambda *s: _rng.normal(s) * 0.05)(D, F) * (D ** -0.5)),
            "w4": _w((lambda *s: _rng.normal(s) * 0.05)(F, D) * (F ** -0.5)),
        }
    _B_in = _B_setup()

    return {
        "A_x": _A_in["x"],
        "A_k_cache": _A_in["k_cache"],
        "A_v_cache": _A_in["v_cache"],
        "A_wq": _A_in["wq"],
        "A_wo": _A_in["wo"],
        "B_x": _B_in["x"],
        "B_w1": _B_in["w1"],
        "B_w2": _B_in["w2"],
        "B_w3": _B_in["w3"],
        "B_w4": _B_in["w4"],
    }

def _fwd_reference(A_x, A_k_cache, A_v_cache, A_wq, A_wo, B_x, B_w1, B_w2, B_w3, B_w4):
    def _A_ref(x, k_cache, v_cache, wq, wo):
        B, Sq, D = x.shape
        Hq, Dh = 32, 128
        Hkv, Sk = k_cache.shape[1], k_cache.shape[2]
        W = min(4096, max(256, Sk // 4))
        rep = Hq // Hkv
        q = (lambda x, *d: x.transpose(*d))((x @ wq).reshape(B, Sq, Hq, Dh), 0, 2, 1, 3)
        k = jnp.repeat(k_cache[:, :, Sk - W:, :], rep, axis=1)
        v = jnp.repeat(v_cache[:, :, Sk - W:, :], rep, axis=1)
        scores = jnp.einsum("bhqd,bhkd->bhqk", q, k) * (Dh ** -0.5)
        p = _softmax(scores, axis=-1)
        o = jnp.einsum("bhqk,bhkd->bhqd", p, v)
        return (lambda x, *d: x.transpose(*d))(o, 0, 2, 1, 3).reshape(B, Sq, Hq * Dh) @ wo

    def _B_ref(x, w1, w2, w3, w4):
        B, S, D = x.shape
        h = _gelu(_layernorm(x, axis=-1) @ w1)
        c = D // 4
        g0 = jnp.pad(h[:, :, 0*c:1*c], ((0, 0), (1, 0), (0, 0)))[:, :S, :]
        g1 = jnp.pad(h[:, :, 1*c:2*c], ((0, 0), (0, 1), (0, 0)))[:, 1:, :]
        g2 = jnp.pad(h[:, :, 2*c:3*c], ((0, 0), (2, 0), (0, 0)))[:, :S, :]
        g3 = jnp.pad(h[:, :, 3*c:   ], ((0, 0), (0, 2), (0, 0)))[:, 2:, :]
        hs = jnp.concatenate([g0, g1, g2, g3], axis=-1) @ w2
        x1 = x + hs
        h2 = _gelu(_layernorm(x1, axis=-1) @ w3) @ w4
        return x1 + h2

    x = A_x
    xn = _layernorm(x, axis=-1)
    s = _A_ref(xn, A_k_cache, A_v_cache, A_wq, A_wo)
    g = _silu(_B_ref(xn, B_w1, B_w2, B_w3, B_w4))
    return x + s * g


def setup_inputs():
    _inp = _fwd_setup_inputs()
    _gk = jax.random.fold_in(jax.random.key(int.from_bytes(__import__("os").urandom(4), "little")), 2**31 - 1)
    _shapes = [[4, 1, 512]]
    _dtypes = ['bfloat16']
    _gks = jax.random.split(_gk, len(_shapes))
    _gs = [jax.random.normal(k, s, dtype=jnp.dtype(d)) * 0.05 for k, s, d in zip(_gks, _shapes, _dtypes)]
    _inp["grad_out"] = _gs[0]
    return _inp

def reference(A_x, A_k_cache, A_v_cache, A_wq, A_wo, B_w3, B_w4, B_x, B_w1, B_w2, grad_out):
    _const = dict(B_x=B_x, B_w1=B_w1, B_w2=B_w2)
    def _f(*_d):
        return _fwd_reference(**{'A_x': _d[0], 'A_k_cache': _d[1], 'A_v_cache': _d[2], 'A_wq': _d[3], 'A_wo': _d[4], 'B_w3': _d[5], 'B_w4': _d[6], **_const})
    _out, _vjp = jax.vjp(_f, A_x, A_k_cache, A_v_cache, A_wq, A_wo, B_w3, B_w4)
    _grads = _vjp(grad_out)
    _out0 = jnp.asarray(_out)
    return (_out0, *[jnp.asarray(_g) for _g in _grads])
```

```python
import math

import jax
import jax.numpy as jnp
from jax import lax
import jax.experimental.pallas as pl
import jax.experimental.pallas.tpu as pltpu

F32 = jnp.float32
BF16 = jnp.bfloat16

_EPS = 1e-5
_GELU_C = math.sqrt(2.0 / math.pi)
_GELU_A = 0.044715
_ROWS = 8

_NN = (((1,), (0,)), ((), ()))
_NT = (((1,), (1,)), ((), ()))
_TN = (((0,), (0,)), ((), ()))


def _dot(a, b, dims):
    return lax.dot_general(a.astype(BF16), b.astype(BF16), dims, preferred_element_type=F32)


def _layernorm(x):
    d = x - jnp.mean(x, axis=-1, keepdims=True)
    rstd = 1.0 / jnp.sqrt(jnp.mean(d * d, axis=-1, keepdims=True) + _EPS)
    return d * rstd, rstd


def _layernorm_bwd(dy, y, rstd):
    return rstd * (
        dy - jnp.mean(dy, axis=-1, keepdims=True) - y * jnp.mean(dy * y, axis=-1, keepdims=True)
    )


def _make_kernel(B, Hkv, rep, Sk, W, Dh, zrows):
    slabs = B * Hkv
    lo = Sk - W
    scale = Dh ** -0.5
    n_zero = lo // zrows
    n_grad = W // zrows
    assert lo % zrows == 0 and W % zrows == 0 and (2 * n_zero) % slabs == 0
    zero_per_slab = 2 * n_zero // slabs

    def kernel(
        x_hbm, g_hbm, k_hbm, v_hbm, wq_hbm, wo_hbm, w3_hbm, w4_hbm,
        out_hbm, dx_hbm, dk_hbm, dv_hbm, dwq_hbm, dwo_hbm, dw3_hbm, dw4_hbm,
        xg_buf, res_buf, pad_buf,
        k_buf, v_buf, dk_buf, dv_buf, zero_buf,
        wq_buf, wo_buf, w3_buf, w4_buf, dwq_buf, dwo_buf, dw3_buf, dw4_buf,
        q_s, do_s, o_s, dq_s,
        in_sems, kv_sem, zero_sems, grad_sem, out_sem,
    ):
        small = [
            pltpu.make_async_copy(x_hbm, xg_buf.at[0], in_sems.at[0]),
            pltpu.make_async_copy(g_hbm, xg_buf.at[1], in_sems.at[1]),
            pltpu.make_async_copy(w3_hbm, w3_buf, in_sems.at[2]),
            pltpu.make_async_copy(w4_hbm, w4_buf, in_sems.at[3]),
            pltpu.make_async_copy(wq_hbm, wq_buf, in_sems.at[4]),
            pltpu.make_async_copy(wo_hbm, wo_buf, in_sems.at[5]),
        ]
        for i, c in enumerate(small):
            c.start(priority=i % 2)
        k_in = pltpu.make_async_copy(k_hbm.at[:, pl.ds(lo, W)], k_buf, kv_sem.at[0])
        v_in = pltpu.make_async_copy(v_hbm.at[:, pl.ds(lo, W)], v_buf, kv_sem.at[1])
        k_in.start(priority=0)
        v_in.start(priority=1)

        zero_buf[...] = jnp.zeros(zero_buf.shape, BF16)
        pad_buf[...] = jnp.zeros(pad_buf.shape, F32)

        small[0].wait()
        small[1].wait()
        pad_buf[0, 0:B, :] = xg_buf[0].astype(F32)
        pad_buf[1, 0:B, :] = xg_buf[1].astype(F32)
        x = pad_buf[0]
        g = pad_buf[1]

        xn, rstd1 = _layernorm(x)
        ln2, rstd2 = _layernorm(xn)
        small[2].wait()
        u = _dot(ln2, w3_buf[...], _NN)
        t = jnp.tanh(_GELU_C * (u + _GELU_A * u * u * u))
        a = 0.5 * u * (1.0 + t)
        small[3].wait()
        y = xn + _dot(a, w4_buf[...], _NN)
        sig = jax.nn.sigmoid(y)
        gate = y * sig
        ds = g * gate

        row = lax.broadcasted_iota(jnp.int32, (_ROWS, Dh), 0)

        def to_slabs(full, ref):
            for h in range(Hkv):
                tiles = [full[:, (h * rep + r) * Dh:(h * rep + r + 1) * Dh] for r in range(rep)]
                for b in range(B):
                    acc = jnp.zeros((_ROWS, Dh), F32)
                    for r in range(rep):
                        acc = jnp.where(row == r, tiles[r][b:b + 1, :], acc)
                    ref[b * Hkv + h] = acc

        def from_slabs(ref):
            cols = []
            for h in range(Hkv):
                tiles = [ref[b * Hkv + h] for b in range(B)]
                for r in range(rep):
                    acc = jnp.zeros((_ROWS, Dh), F32)
                    for b in range(B):
                        acc = jnp.where(row == b, tiles[b][r:r + 1, :], acc)
                    cols.append(acc)
            return jnp.concatenate(cols, axis=1)

        small[4].wait()
        to_slabs(_dot(xn, wq_buf[...], _NN), q_s)
        small[5].wait()
        to_slabs(_dot(ds, wo_buf[...], _NT), do_s)

        k_in.wait()
        v_in.wait()

        def zero_copy(i, dst, slot):
            r0 = pl.multiple_of(i * zrows, zrows)
            return pltpu.make_async_copy(zero_buf, dst.at[:, pl.ds(r0, zrows)], zero_sems.at[slot])

        def start_zeros(j):
            for half, (dst, p) in enumerate(((dk_hbm, 0), (dv_hbm, 1))):
                @pl.when((j < slabs // 2) if half == 0 else (j >= slabs // 2))
                def _():
                    jj = j - half * (slabs // 2)
                    for i in range(zero_per_slab):
                        zero_copy(jj * zero_per_slab + i, dst, j % 2).start(priority=i % 2)

        def wait_zeros(slot):
            for _ in range(zero_per_slab):
                zero_copy(0, dk_hbm, slot).wait()

        def attend(j):
            q = q_s[j]
            do = do_s[j]
            k = k_buf[j]
            v = v_buf[j]
            s = _dot(q, k, _NT) * scale
            e = jnp.exp(s - jnp.max(s, axis=-1, keepdims=True))
            p = e / jnp.sum(e, axis=-1, keepdims=True)
            dp = _dot(do, v, _NT)
            dsc = p * (dp - jnp.sum(p * dp, axis=-1, keepdims=True)) * scale
            o_s[j] = _dot(p, v, _NN)
            dq_s[j] = _dot(dsc, k, _NN)
            zero = jnp.zeros((_ROWS, Dh), F32)
            rhs = jnp.concatenate(
                [jnp.concatenate([do, zero], axis=1), jnp.concatenate([zero, q], axis=1)], axis=0
            )
            dvk = _dot(jnp.concatenate([p, dsc], axis=0), rhs, _TN).astype(BF16)
            dv_buf[j] = dvk[:, :Dh]
            dk_buf[j] = dvk[:, Dh:]

        start_zeros(0)

        def body(j, carry):
            @pl.when(j + 1 < slabs)
            def _():
                start_zeros(j + 1)

            attend(j)

            @pl.when(j + 1 < slabs)
            def _():
                wait_zeros(j % 2)

            return carry

        lax.fori_loop(0, slabs, body, 0)

        for i in range(n_grad):
            rows = pl.ds(i * zrows, zrows)
            pltpu.make_async_copy(dk_buf.at[:, rows], dk_hbm.at[:, pl.ds(lo + i * zrows, zrows)], grad_sem).start(priority=i % 2)
        for i in range(n_grad):
            rows = pl.ds(i * zrows, zrows)
            pltpu.make_async_copy(dv_buf.at[:, rows], dv_hbm.at[:, pl.ds(lo + i * zrows, zrows)], grad_sem).start(priority=i % 2)

        o = from_slabs(o_s)
        dq = from_slabs(dq_s)
        s = _dot(o, wo_buf[...], _NN)
        dy = g * s * sig * (1.0 + y * (1.0 - sig))
        da = _dot(dy, w4_buf[...], _NT)
        du = da * (0.5 * (1.0 + t) + 0.5 * u * (1.0 - t * t) * _GELU_C * (1.0 + 3.0 * _GELU_A * u * u))
        dxn = dy + _layernorm_bwd(_dot(du, w3_buf[...], _NT), ln2, rstd2) + _dot(dq, wq_buf[...], _NT)
        res_buf[0] = (x + s * gate)[0:B].astype(BF16)
        res_buf[1] = (g + _layernorm_bwd(dxn, xn, rstd1))[0:B].astype(BF16)
        dwq_buf[...] = _dot(xn, dq, _TN).astype(BF16)
        dwo_buf[...] = _dot(o, ds, _TN).astype(BF16)
        dw3_buf[...] = _dot(ln2, du, _TN).astype(BF16)
        dw4_buf[...] = _dot(a, dy, _TN).astype(BF16)

        tail = [
            pltpu.make_async_copy(res_buf.at[0], out_hbm, out_sem),
            pltpu.make_async_copy(res_buf.at[1], dx_hbm, out_sem),
            pltpu.make_async_copy(dwq_buf, dwq_hbm, out_sem),
            pltpu.make_async_copy(dwo_buf, dwo_hbm, out_sem),
            pltpu.make_async_copy(dw3_buf, dw3_hbm, out_sem),
            pltpu.make_async_copy(dw4_buf, dw4_hbm, out_sem),
        ]
        for i, c in enumerate(tail):
            c.start(priority=i % 2)

        wait_zeros((slabs - 1) % 2)
        pltpu.make_async_copy(dk_buf, dk_buf, grad_sem).wait()
        pltpu.make_async_copy(dv_buf, dv_buf, grad_sem).wait()
        for c in tail:
            c.wait()

    return kernel


@jax.jit
def pallas_recurrent_scan__sliding_block_cached__mixer_s_mlp__decode_kernel(
    A_x: jax.Array,
    A_k_cache: jax.Array,
    A_v_cache: jax.Array,
    A_wq: jax.Array,
    A_wo: jax.Array,
    B_x: jax.Array,
    B_w1: jax.Array,
    B_w2: jax.Array,
    B_w3: jax.Array,
    B_w4: jax.Array,
    grad_out: jax.Array,
):
    del B_x, B_w1, B_w2
    B, S, D = A_x.shape
    _, Hkv, Sk, Dh = A_k_cache.shape
    HD = A_wq.shape[1]
    F = B_w3.shape[1]
    assert S == 1 and B <= _ROWS
    rep = HD // Dh // Hkv
    W = min(4096, max(256, Sk // 4))
    slabs = B * Hkv
    zrows = 128

    hbm = pl.BlockSpec(memory_space=pltpu.HBM)
    sds = jax.ShapeDtypeStruct
    out, dx, dk, dv, dwq, dwo, dw3, dw4 = pl.pallas_call(
        _make_kernel(B, Hkv, rep, Sk, W, Dh, zrows),
        in_specs=[hbm] * 8,
        out_specs=[hbm] * 8,
        out_shape=[
            sds((B, D), BF16), sds((B, D), BF16),
            sds((slabs, Sk, Dh), BF16), sds((slabs, Sk, Dh), BF16),
            sds((D, HD), BF16), sds((HD, D), BF16), sds((D, F), BF16), sds((F, D), BF16),
        ],
        scratch_shapes=[
            pltpu.VMEM((2, B, D), BF16), pltpu.VMEM((2, B, D), BF16), pltpu.VMEM((2, _ROWS, D), F32),
            pltpu.VMEM((slabs, W, Dh), BF16), pltpu.VMEM((slabs, W, Dh), BF16),
            pltpu.VMEM((slabs, W, Dh), BF16), pltpu.VMEM((slabs, W, Dh), BF16),
            pltpu.VMEM((slabs, zrows, Dh), BF16),
            pltpu.VMEM((D, HD), BF16), pltpu.VMEM((HD, D), BF16),
            pltpu.VMEM((D, F), BF16), pltpu.VMEM((F, D), BF16),
            pltpu.VMEM((D, HD), BF16), pltpu.VMEM((HD, D), BF16),
            pltpu.VMEM((D, F), BF16), pltpu.VMEM((F, D), BF16),
            pltpu.VMEM((slabs, _ROWS, Dh), F32), pltpu.VMEM((slabs, _ROWS, Dh), F32),
            pltpu.VMEM((slabs, _ROWS, Dh), F32), pltpu.VMEM((slabs, _ROWS, Dh), F32),
            pltpu.SemaphoreType.DMA((6,)), pltpu.SemaphoreType.DMA((2,)), pltpu.SemaphoreType.DMA((2,)),
            pltpu.SemaphoreType.DMA, pltpu.SemaphoreType.DMA,
        ],
        compiler_params=pltpu.CompilerParams(vmem_limit_bytes=120 << 20),
        name="window_attn_mixer_fwd_bwd",
    )(
        A_x.reshape(B, D), grad_out.reshape(B, D),
        A_k_cache.reshape(slabs, Sk, Dh), A_v_cache.reshape(slabs, Sk, Dh),
        A_wq, A_wo, B_w3, B_w4,
    )
    return (
        out.reshape(B, S, D), dx.reshape(B, S, D),
        dk.reshape(B, Hkv, Sk, Dh), dv.reshape(B, Hkv, Sk, Dh),
        dwq, dwo, dw3, dw4,
    )
```

```python
import math

import jax
import jax.numpy as jnp
from jax import lax
import jax.experimental.pallas as pl
import jax.experimental.pallas.tpu as pltpu

F32 = jnp.float32
BF16 = jnp.bfloat16

_EPS = 1e-5
_GELU_C = math.sqrt(2.0 / math.pi)
_GELU_A = 0.044715

_ROWS = 8
_TILE = 8

_READ_SLABS = 4
_READ_ROWS = 32
_READ_TAIL = 14
_WRITE_SLABS = 8
_WRITE_ROWS = 104

_NN = (((1,), (0,)), ((), ()))
_NT = (((1,), (1,)), ((), ()))
_TN = (((0,), (0,)), ((), ()))


def _dot(a, b, dims):
    return lax.dot_general(a.astype(BF16), b.astype(BF16), dims, preferred_element_type=F32)


def _layernorm(x):
    d = x - jnp.mean(x, axis=-1, keepdims=True)
    rstd = 1.0 / jnp.sqrt(jnp.mean(d * d, axis=-1, keepdims=True) + _EPS)
    return d * rstd, rstd


def _layernorm_bwd(dy, y, rstd):
    return rstd * (
        dy - jnp.mean(dy, axis=-1, keepdims=True) - y * jnp.mean(dy * y, axis=-1, keepdims=True)
    )


def _loop(lo, hi, body):
    def step(i, carry):
        body(i)
        return carry

    lax.fori_loop(lo, hi, step, 0)


def _block(i, n):
    return pl.ds(pl.multiple_of(i * n, _TILE), n)


def _matrix(ref):
    return ref[...].reshape(ref.shape[0] * ref.shape[1], ref.shape[2])


def _kernel(
    x_hbm, g_hbm, k_hbm, v_hbm, wq_hbm, wo_hbm, w3_hbm, w4_hbm,
    out_hbm, dx_hbm, dk_hbm, dv_hbm, dwq_hbm, dwo_hbm, dw3_hbm, dw4_hbm,
    xg_buf, pad_buf, res_buf,
    k_buf, v_buf, dk_buf, dv_buf, zero_buf,
    wq_buf, wo_buf, w3_buf, w4_buf, dwq_buf, dwo_buf, dw3_buf, dw4_buf,
    q_buf, do_buf, o_buf, dq_buf,
    sem, tail_sem,
):
    batch = x_hbm.shape[0]
    slabs, window, dh = k_buf.shape
    first = k_hbm.shape[1] - window
    kv_heads = slabs // batch
    rep = wq_hbm.shape[2] // (kv_heads * dh)
    groups = dk_hbm.shape[1]
    scale = dh ** -0.5

    def start(src, dst, priority=0, sem=sem):
        pltpu.make_async_copy(src, dst, sem).start(priority=priority)

    def wait_filled(ref, sem=sem):
        pltpu.make_async_copy(ref, ref, sem).wait()

    def read_pair(wide_hbm, wide_buf, tall_hbm, tall_buf):
        steps = tall_hbm.shape[1] // _TILE
        per_row = steps // (wide_hbm.shape[1] // _TILE)
        cols = wide_hbm.shape[2] // per_row

        def step(i):
            r = _block(lax.div(i, per_row), _TILE)
            c = pl.ds(pl.multiple_of(lax.rem(i, per_row) * cols, cols), cols)
            start(wide_hbm.at[:, r, c], wide_buf.at[:, r, c], 0)
            r = _block(i, _TILE)
            start(tall_hbm.at[:, r], tall_buf.at[:, r], 1)

        _loop(0, steps, step)

    read_pair(wq_hbm, wq_buf, wo_hbm, wo_buf)
    start(x_hbm, xg_buf.at[0], 0)
    start(g_hbm, xg_buf.at[1], 1)
    read_pair(w3_hbm, w3_buf, w4_hbm, w4_buf)

    per_slab = window // _READ_ROWS
    kv_reads = slabs // _READ_SLABS * per_slab

    def read_kv(i, sem):
        b = pl.ds(lax.div(i, per_slab) * _READ_SLABS, _READ_SLABS)
        r = pl.multiple_of(lax.rem(i, per_slab) * _READ_ROWS, _READ_ROWS)
        src, dst = pl.ds(first + r, _READ_ROWS), pl.ds(r, _READ_ROWS)
        start(k_hbm.at[b, src], k_buf.at[b, dst], 0, sem)
        start(v_hbm.at[b, src], v_buf.at[b, dst], 1, sem)

    _loop(0, kv_reads - _READ_TAIL, lambda i: read_kv(i, sem))
    _loop(kv_reads - _READ_TAIL, kv_reads, lambda i: read_kv(i, tail_sem))

    zero_buf[...] = jnp.zeros(zero_buf.shape, BF16)
    pad_buf[...] = jnp.zeros(pad_buf.shape, F32)

    last = pl.ds(slabs - _READ_SLABS, _READ_SLABS)
    early = window - _READ_TAIL * _READ_ROWS
    for buf in (xg_buf, wq_buf, wo_buf, w3_buf, w4_buf):
        wait_filled(buf)
    for buf in (k_buf, v_buf):
        wait_filled(buf.at[pl.ds(0, slabs - _READ_SLABS)])
        wait_filled(buf.at[last, pl.ds(0, early)])

    def sweep(rows, write):
        full, rest = divmod(rows, _WRITE_ROWS)
        _loop(0, full, lambda i: write(pl.multiple_of(i * _WRITE_ROWS, _TILE), _WRITE_ROWS))
        if rest:
            write(full * _WRITE_ROWS, rest)

    def write_zeros(dst, group):
        sweep(first, lambda r, n: start(zero_buf.at[:, pl.ds(0, n)], dst.at[:, group, pl.ds(r, n)]))

    write_zeros(dk_hbm, 0)
    for buf in (k_buf, v_buf):
        wait_filled(buf.at[last, pl.ds(early, window - early)], tail_sem)

    pad_buf[0, 0:batch, :] = xg_buf[0].astype(F32)
    pad_buf[1, 0:batch, :] = xg_buf[1].astype(F32)
    x = pad_buf[0]
    g = pad_buf[1]

    xn, rstd1 = _layernorm(x)
    ln2, rstd2 = _layernorm(xn)
    u = _dot(ln2, _matrix(w3_buf), _NN)
    t = jnp.tanh(_GELU_C * (u + _GELU_A * u * u * u))
    a = 0.5 * u * (1.0 + t)
    y = xn + _dot(a, _matrix(w4_buf), _NN)
    sig = jax.nn.sigmoid(y)
    gate = y * sig
    ds = g * gate

    row = lax.broadcasted_iota(jnp.int32, (_ROWS, dh), 0)

    def to_slabs(full, ref):
        for h in range(kv_heads):
            tiles = [full[:, (h * rep + r) * dh:(h * rep + r + 1) * dh] for r in range(rep)]
            for b in range(batch):
                acc = jnp.zeros((_ROWS, dh), F32)
                for r in range(rep):
                    acc = jnp.where(row == r, tiles[r][b:b + 1, :], acc)
                ref[b * kv_heads + h] = acc

    def from_slabs(ref):
        cols = []
        for h in range(kv_heads):
            tiles = [ref[b * kv_heads + h] for b in range(batch)]
            for r in range(rep):
                acc = jnp.zeros((_ROWS, dh), F32)
                for b in range(batch):
                    acc = jnp.where(row == b, tiles[b][r:r + 1, :], acc)
                cols.append(acc)
        return jnp.concatenate(cols, axis=1)

    to_slabs(_dot(xn, _matrix(wq_buf), _NN), q_buf)
    to_slabs(_dot(ds, _matrix(wo_buf), _NT), do_buf)

    def attend(j):
        q, do, k, v = q_buf[j], do_buf[j], k_buf[j], v_buf[j]
        s = _dot(q, k, _NT) * scale
        e = jnp.exp(s - jnp.max(s, axis=-1, keepdims=True))
        p = e / jnp.sum(e, axis=-1, keepdims=True)
        dp = _dot(do, v, _NT)
        dsc = p * (dp - jnp.sum(p * dp, axis=-1, keepdims=True)) * scale
        o_buf[j] = _dot(p, v, _NN)
        dq_buf[j] = _dot(dsc, k, _NN)
        zero = jnp.zeros((_ROWS, dh), F32)
        rhs = jnp.concatenate(
            [jnp.concatenate([do, zero], axis=1), jnp.concatenate([zero, q], axis=1)], axis=0
        )
        dvk = _dot(jnp.concatenate([p, dsc], axis=0), rhs, _TN).astype(BF16)
        dv_buf[lax.div(j, groups), lax.rem(j, groups)] = dvk[:, :dh]
        dk_buf[lax.div(j, groups), lax.rem(j, groups)] = dvk[:, dh:]

    per_sweep = slabs // (2 * groups)

    def step(i):
        @pl.when(i + 1 < groups)
        def _():
            write_zeros(dk_hbm, i + 1)

        @pl.when(jnp.logical_and(i + 1 >= groups, i + 1 < 2 * groups))
        def _():
            write_zeros(dv_hbm, i + 1 - groups)

        _loop(i * per_sweep, (i + 1) * per_sweep, attend)

    _loop(0, 2 * groups, step)

    def write_grads(src, dst):
        _loop(0, groups, lambda group: sweep(window, lambda r, n: start(
            src.at[:, group, pl.ds(r, n)], dst.at[:, group, pl.ds(first + r, n)])))

    write_grads(dk_buf, dk_hbm)
    write_grads(dv_buf, dv_hbm)

    o = from_slabs(o_buf)
    dq = from_slabs(dq_buf)
    s = _dot(o, _matrix(wo_buf), _NN)
    dy = g * s * sig * (1.0 + y * (1.0 - sig))
    da = _dot(dy, _matrix(w4_buf), _NT)
    du = da * (0.5 * (1.0 + t) + 0.5 * u * (1.0 - t * t) * _GELU_C * (1.0 + 3.0 * _GELU_A * u * u))
    dxn = (
        dy
        + _layernorm_bwd(_dot(du, _matrix(w3_buf), _NT), ln2, rstd2)
        + _dot(dq, _matrix(wq_buf), _NT)
    )
    res_buf[0] = (x + s * gate)[0:batch].astype(BF16)
    res_buf[1] = (g + _layernorm_bwd(dxn, xn, rstd1))[0:batch].astype(BF16)
    for ref, lhs, rhs in ((dwq_buf, xn, dq), (dwo_buf, o, ds), (dw3_buf, ln2, du), (dw4_buf, a, dy)):
        ref[...] = _dot(lhs, rhs, _TN).astype(BF16).reshape(ref.shape)

    start(res_buf.at[0], out_hbm)
    start(res_buf.at[1], dx_hbm)

    def write_part(src, dst, *index):
        index = (slice(None),) + index
        start(src.at[index], dst.at[index])

    tall = 4 * _TILE

    def write_weights(i):
        half = dwq_buf.shape[2] // 2
        cols = pl.ds(pl.multiple_of(lax.rem(i, 2) * half, half), half)
        write_part(dwq_buf, dwq_hbm, _block(lax.div(i, 2), _TILE), cols)

        @pl.when(i < dw3_buf.shape[1] // _TILE)
        def _():
            write_part(dw3_buf, dw3_hbm, _block(i, _TILE))

        write_part(dwo_buf, dwo_hbm, _block(i, tall))

        @pl.when(i < dw4_buf.shape[1] // tall)
        def _():
            write_part(dw4_buf, dw4_hbm, _block(i, tall))

    steps = dwo_buf.shape[1] // tall
    assert steps == 2 * dwq_buf.shape[1] // _TILE
    assert dw3_buf.shape[1] // _TILE <= steps and dw4_buf.shape[1] // tall <= steps
    _loop(0, steps, write_weights)

    for ref in (out_hbm, dx_hbm, dk_hbm, dv_hbm, dwq_hbm, dwo_hbm, dw3_hbm, dw4_hbm):
        wait_filled(ref)


@jax.jit
def pallas_recurrent_scan__sliding_block_cached__mixer_s_mlp__decode_kernel(
    A_x: jax.Array,
    A_k_cache: jax.Array,
    A_v_cache: jax.Array,
    A_wq: jax.Array,
    A_wo: jax.Array,
    B_x: jax.Array,
    B_w1: jax.Array,
    B_w2: jax.Array,
    B_w3: jax.Array,
    B_w4: jax.Array,
    grad_out: jax.Array,
):
    del B_x, B_w1, B_w2
    batch, seq, dim = A_x.shape
    _, kv_heads, keys, dh = A_k_cache.shape
    assert seq == 1 and batch <= _ROWS
    window = min(4096, max(256, keys // 4))
    slabs = batch * kv_heads
    groups = slabs // _WRITE_SLABS

    def split(w, n):
        return (n, w.shape[0] // n, w.shape[1])

    weights = (A_wq, A_wo, B_w3, B_w4)
    read_shapes = [split(w, n) for w, n in zip(weights, (4, 4, 8, 4))]
    write_shapes = [split(w, n) for w, n in zip(weights, (2, 2, 1, 1))]

    hbm = pl.BlockSpec(memory_space=pltpu.HBM)
    out, dx, dk, dv, *dws = pl.pallas_call(
        _kernel,
        in_specs=[hbm] * 8,
        out_specs=[hbm] * 8,
        out_shape=[
            jax.ShapeDtypeStruct(shape, BF16)
            for shape in [(batch, dim)] * 2 + [(_WRITE_SLABS, groups, keys, dh)] * 2 + write_shapes
        ],
        scratch_shapes=[
            pltpu.VMEM((2, batch, dim), BF16),
            pltpu.VMEM((2, _ROWS, dim), F32),
            pltpu.VMEM((2, batch, dim), BF16),
            *[pltpu.VMEM((slabs, window, dh), BF16)] * 2,
            *[pltpu.VMEM((_WRITE_SLABS, groups, window, dh), BF16)] * 2,
            pltpu.VMEM((_WRITE_SLABS, _WRITE_ROWS, dh), BF16),
            *[pltpu.VMEM(shape, BF16) for shape in read_shapes + write_shapes],
            *[pltpu.VMEM((slabs, _ROWS, dh), F32)] * 4,
            *[pltpu.SemaphoreType.DMA] * 2,
        ],
        compiler_params=pltpu.CompilerParams(vmem_limit_bytes=120 << 20),
        name="window_attention_mixer_fwd_bwd",
    )(
        A_x.reshape(batch, dim),
        grad_out.reshape(batch, dim),
        A_k_cache.reshape(slabs, keys, dh),
        A_v_cache.reshape(slabs, keys, dh),
        *[w.reshape(shape) for w, shape in zip(weights, read_shapes)],
    )
    return (
        out.reshape(A_x.shape),
        dx.reshape(A_x.shape),
        dk.reshape(A_k_cache.shape),
        dv.reshape(A_v_cache.shape),
        *[dw.reshape(w.shape) for dw, w in zip(dws, weights)],
    )
```

```python
import math

import jax
import jax.numpy as jnp
from jax import lax
import jax.experimental.pallas as pl
import jax.experimental.pallas.tpu as pltpu

F32 = jnp.float32
BF16 = jnp.bfloat16

_EPS = 1e-5
_GELU_C = math.sqrt(2.0 / math.pi)
_GELU_A = 0.044715

_ROWS = 8
_TILE = 8

_READ_SLABS = 8
_READ_ROWS = 16
_READ_TAIL = 14
_READ_COLS = 256
_WRITE_SLABS = 8
_WRITE_ROWS = 112

_NN = (((1,), (0,)), ((), ()))
_NT = (((1,), (1,)), ((), ()))
_TN = (((0,), (0,)), ((), ()))


def _dot(a, b, dims):
    return lax.dot_general(a.astype(BF16), b.astype(BF16), dims, preferred_element_type=F32)


def _layernorm(x):
    d = x - jnp.mean(x, axis=-1, keepdims=True)
    rstd = 1.0 / jnp.sqrt(jnp.mean(d * d, axis=-1, keepdims=True) + _EPS)
    return d * rstd, rstd


def _layernorm_bwd(dy, y, rstd):
    return rstd * (
        dy - jnp.mean(dy, axis=-1, keepdims=True) - y * jnp.mean(dy * y, axis=-1, keepdims=True)
    )


def _loop(lo, hi, body):
    def step(i, carry):
        body(i)
        return carry

    lax.fori_loop(lo, hi, step, 0)


def _block(i, n):
    return pl.ds(pl.multiple_of(i * n, n), n)


def _matrix(ref):
    return ref[...].reshape(ref.shape[0] * ref.shape[1], ref.shape[2])


def _kernel(
    x_hbm, g_hbm, k_hbm, v_hbm, wq_hbm, wo_hbm, w3_hbm, w4_hbm,
    out_hbm, dx_hbm, dk_hbm, dv_hbm, dwq_hbm, dwo_hbm, dw3_hbm, dw4_hbm,
    xg_buf, pad_buf, res_buf,
    k_buf, v_buf, dk_buf, dv_buf, zero_buf,
    wq_buf, wo_buf, w3_buf, w4_buf, dwq_buf, dwo_buf, dw3_buf, dw4_buf,
    q_buf, do_buf, o_buf, dq_buf,
    sem, tail_sem,
):
    batch = x_hbm.shape[0]
    slabs, window, dh = k_buf.shape
    first = k_hbm.shape[1] - window
    kv_heads = slabs // batch
    rep = wq_hbm.shape[2] // (kv_heads * dh)
    groups = dk_hbm.shape[1]
    scale = dh ** -0.5

    def start(src, dst, priority=0, sem=sem):
        pltpu.make_async_copy(src, dst, sem).start(priority=priority)

    def wait_filled(ref, sem=sem):
        pltpu.make_async_copy(ref, ref, sem).wait()

    start(x_hbm, xg_buf.at[0], 0)
    start(g_hbm, xg_buf.at[1], 1)

    def read_weights(wide_hbm, wide_buf, tall_hbm, tall_buf):
        per_row = wide_hbm.shape[2] // _READ_COLS
        steps = tall_hbm.shape[1] // _TILE
        per_step = wide_hbm.shape[1] // _TILE * per_row // steps
        assert steps * per_step == wide_hbm.shape[1] // _TILE * per_row

        def step(i):
            for n in range(per_step):
                r = _block(lax.div(i * per_step + n, per_row), _TILE)
                c = _block(lax.rem(i * per_step + n, per_row), _READ_COLS)
                start(wide_hbm.at[:, r, c], wide_buf.at[:, r, c], 0)
            start(tall_hbm.at[:, _block(i, _TILE)], tall_buf.at[:, _block(i, _TILE)], 1)

        _loop(0, steps, step)

    read_weights(w3_hbm, w3_buf, w4_hbm, w4_buf)
    read_weights(wq_hbm, wq_buf, wo_hbm, wo_buf)

    per_slab = window // _READ_ROWS
    kv_reads = slabs // _READ_SLABS * per_slab

    def read_kv(i, sem):
        b = pl.ds(lax.div(i, per_slab) * _READ_SLABS, _READ_SLABS)
        r = pl.multiple_of(lax.rem(i, per_slab) * _READ_ROWS, _READ_ROWS)
        src, dst = pl.ds(first + r, _READ_ROWS), pl.ds(r, _READ_ROWS)
        start(k_hbm.at[b, src], k_buf.at[b, dst], 0, sem)
        start(v_hbm.at[b, src], v_buf.at[b, dst], 1, sem)

    _loop(0, kv_reads - _READ_TAIL, lambda i: read_kv(i, sem))
    _loop(kv_reads - _READ_TAIL, kv_reads, lambda i: read_kv(i, tail_sem))

    zero_buf[...] = jnp.zeros(zero_buf.shape, BF16)
    pad_buf[...] = jnp.zeros(pad_buf.shape, F32)

    last = pl.ds(slabs - _READ_SLABS, _READ_SLABS)
    early = window - _READ_TAIL * _READ_ROWS
    for buf in (xg_buf, wq_buf, wo_buf, w3_buf, w4_buf):
        wait_filled(buf)
    for buf in (k_buf, v_buf):
        wait_filled(buf.at[pl.ds(0, slabs - _READ_SLABS)])
        wait_filled(buf.at[last, pl.ds(0, early)])

    def sweep(rows, write):
        full, rest = divmod(rows, _WRITE_ROWS)
        _loop(0, full, lambda i: write(pl.multiple_of(i * _WRITE_ROWS, _TILE), _WRITE_ROWS))
        if rest:
            write(full * _WRITE_ROWS, rest)

    def write_zeros(dst, group):
        sweep(first, lambda r, n: start(zero_buf.at[:, pl.ds(0, n)], dst.at[:, group, pl.ds(r, n)]))

    write_zeros(dk_hbm, 0)
    for buf in (k_buf, v_buf):
        wait_filled(buf.at[last, pl.ds(early, window - early)], tail_sem)

    pad_buf[0, 0:batch, :] = xg_buf[0].astype(F32)
    pad_buf[1, 0:batch, :] = xg_buf[1].astype(F32)
    x = pad_buf[0]
    g = pad_buf[1]

    xn, rstd1 = _layernorm(x)
    ln2, rstd2 = _layernorm(xn)
    u = _dot(ln2, _matrix(w3_buf), _NN)
    t = jnp.tanh(_GELU_C * (u + _GELU_A * u * u * u))
    a = 0.5 * u * (1.0 + t)
    y = xn + _dot(a, _matrix(w4_buf), _NN)
    sig = jax.nn.sigmoid(y)
    gate = y * sig
    ds = g * gate

    row = lax.broadcasted_iota(jnp.int32, (_ROWS, dh), 0)

    def to_slabs(full, ref):
        for h in range(kv_heads):
            tiles = [full[:, (h * rep + r) * dh:(h * rep + r + 1) * dh] for r in range(rep)]
            for b in range(batch):
                acc = jnp.zeros((_ROWS, dh), F32)
                for r in range(rep):
                    acc = jnp.where(row == r, tiles[r][b:b + 1, :], acc)
                ref[b * kv_heads + h] = acc

    def from_slabs(ref):
        cols = []
        for h in range(kv_heads):
            tiles = [ref[b * kv_heads + h] for b in range(batch)]
            for r in range(rep):
                acc = jnp.zeros((_ROWS, dh), F32)
                for b in range(batch):
                    acc = jnp.where(row == b, tiles[b][r:r + 1, :], acc)
                cols.append(acc)
        return jnp.concatenate(cols, axis=1)

    to_slabs(_dot(xn, _matrix(wq_buf), _NN), q_buf)
    to_slabs(_dot(ds, _matrix(wo_buf), _NT), do_buf)

    def attend(j):
        q, do, k, v = q_buf[j], do_buf[j], k_buf[j], v_buf[j]
        s = _dot(q, k, _NT) * scale
        e = jnp.exp(s - jnp.max(s, axis=-1, keepdims=True))
        p = e / jnp.sum(e, axis=-1, keepdims=True)
        dp = _dot(do, v, _NT)
        dsc = p * (dp - jnp.sum(p * dp, axis=-1, keepdims=True)) * scale
        o_buf[j] = _dot(p, v, _NN)
        dq_buf[j] = _dot(dsc, k, _NN)
        zero = jnp.zeros((_ROWS, dh), F32)
        rhs = jnp.concatenate(
            [jnp.concatenate([do, zero], axis=1), jnp.concatenate([zero, q], axis=1)], axis=0
        )
        dvk = _dot(jnp.concatenate([p, dsc], axis=0), rhs, _TN).astype(BF16)
        dv_buf[lax.div(j, groups), lax.rem(j, groups)] = dvk[:, :dh]
        dk_buf[lax.div(j, groups), lax.rem(j, groups)] = dvk[:, dh:]

    per_sweep = slabs // (2 * groups)

    def step(i):
        @pl.when(i + 1 < groups)
        def _():
            write_zeros(dk_hbm, i + 1)

        @pl.when(jnp.logical_and(i + 1 >= groups, i + 1 < 2 * groups))
        def _():
            write_zeros(dv_hbm, i + 1 - groups)

        _loop(i * per_sweep, (i + 1) * per_sweep, attend)

    _loop(0, 2 * groups, step)

    def write_grads(src, dst):
        _loop(0, groups, lambda group: sweep(window, lambda r, n: start(
            src.at[:, group, pl.ds(r, n)], dst.at[:, group, pl.ds(first + r, n)])))

    write_grads(dk_buf, dk_hbm)
    write_grads(dv_buf, dv_hbm)

    o = from_slabs(o_buf)
    dq = from_slabs(dq_buf)
    s = _dot(o, _matrix(wo_buf), _NN)
    dy = g * s * sig * (1.0 + y * (1.0 - sig))
    da = _dot(dy, _matrix(w4_buf), _NT)
    du = da * (0.5 * (1.0 + t) + 0.5 * u * (1.0 - t * t) * _GELU_C * (1.0 + 3.0 * _GELU_A * u * u))
    dxn = (
        dy
        + _layernorm_bwd(_dot(du, _matrix(w3_buf), _NT), ln2, rstd2)
        + _dot(dq, _matrix(wq_buf), _NT)
    )
    res_buf[0] = (x + s * gate)[0:batch].astype(BF16)
    res_buf[1] = (g + _layernorm_bwd(dxn, xn, rstd1))[0:batch].astype(BF16)
    for ref, lhs, rhs in ((dwq_buf, xn, dq), (dwo_buf, o, ds), (dw3_buf, ln2, du), (dw4_buf, a, dy)):
        ref[...] = _dot(lhs, rhs, _TN).astype(BF16).reshape(ref.shape)

    start(res_buf.at[0], out_hbm)
    start(res_buf.at[1], dx_hbm)

    def write_part(src, dst, *index):
        index = (slice(None),) + index
        start(src.at[index], dst.at[index])

    tall = 4 * _TILE

    def write_weights(i):
        cols = _block(lax.rem(i, 2), dwq_buf.shape[2] // 2)
        write_part(dwq_buf, dwq_hbm, _block(lax.div(i, 2), _TILE), cols)

        @pl.when(i < dw3_buf.shape[1] // _TILE)
        def _():
            write_part(dw3_buf, dw3_hbm, _block(i, _TILE))

        write_part(dwo_buf, dwo_hbm, _block(i, tall))

        @pl.when(i < dw4_buf.shape[1] // tall)
        def _():
            write_part(dw4_buf, dw4_hbm, _block(i, tall))

    steps = dwo_buf.shape[1] // tall
    assert steps == 2 * dwq_buf.shape[1] // _TILE
    assert dw3_buf.shape[1] // _TILE <= steps and dw4_buf.shape[1] // tall <= steps
    _loop(0, steps, write_weights)

    for ref in (out_hbm, dx_hbm, dk_hbm, dv_hbm, dwq_hbm, dwo_hbm, dw3_hbm, dw4_hbm):
        wait_filled(ref)


@jax.jit
def pallas_recurrent_scan__sliding_block_cached__mixer_s_mlp__decode_kernel(
    A_x: jax.Array,
    A_k_cache: jax.Array,
    A_v_cache: jax.Array,
    A_wq: jax.Array,
    A_wo: jax.Array,
    B_x: jax.Array,
    B_w1: jax.Array,
    B_w2: jax.Array,
    B_w3: jax.Array,
    B_w4: jax.Array,
    grad_out: jax.Array,
):
    del B_x, B_w1, B_w2
    batch, seq, dim = A_x.shape
    _, kv_heads, keys, dh = A_k_cache.shape
    assert seq == 1 and batch <= _ROWS
    window = min(4096, max(256, keys // 4))
    slabs = batch * kv_heads
    groups = slabs // _WRITE_SLABS

    def split(w, n):
        return (n, w.shape[0] // n, w.shape[1])

    weights = (A_wq, A_wo, B_w3, B_w4)
    read_shapes = [split(w, 4) for w in weights]
    write_shapes = [split(w, n) for w, n in zip(weights, (2, 2, 1, 1))]

    hbm = pl.BlockSpec(memory_space=pltpu.HBM)
    out, dx, dk, dv, *dws = pl.pallas_call(
        _kernel,
        in_specs=[hbm] * 8,
        out_specs=[hbm] * 8,
        out_shape=[
            jax.ShapeDtypeStruct(shape, BF16)
            for shape in [(batch, dim)] * 2 + [(_WRITE_SLABS, groups, keys, dh)] * 2 + write_shapes
        ],
        scratch_shapes=[
            pltpu.VMEM((2, batch, dim), BF16),
            pltpu.VMEM((2, _ROWS, dim), F32),
            pltpu.VMEM((2, batch, dim), BF16),
            *[pltpu.VMEM((slabs, window, dh), BF16)] * 2,
            *[pltpu.VMEM((_WRITE_SLABS, groups, window, dh), BF16)] * 2,
            pltpu.VMEM((_WRITE_SLABS, _WRITE_ROWS, dh), BF16),
            *[pltpu.VMEM(shape, BF16) for shape in read_shapes + write_shapes],
            *[pltpu.VMEM((slabs, _ROWS, dh), F32)] * 4,
            *[pltpu.SemaphoreType.DMA] * 2,
        ],
        compiler_params=pltpu.CompilerParams(vmem_limit_bytes=120 << 20),
        name="window_attention_mixer_fwd_bwd",
    )(
        A_x.reshape(batch, dim),
        grad_out.reshape(batch, dim),
        A_k_cache.reshape(slabs, keys, dh),
        A_v_cache.reshape(slabs, keys, dh),
        *[w.reshape(shape) for w, shape in zip(weights, read_shapes)],
    )
    return (
        out.reshape(A_x.shape),
        dx.reshape(A_x.shape),
        dk.reshape(A_k_cache.shape),
        dv.reshape(A_v_cache.shape),
        *[dw.reshape(w.shape) for dw, w in zip(dws, weights)],
    )
```

```python
import math

import jax
import jax.numpy as jnp
from jax import lax
import jax.experimental.pallas as pl
import jax.experimental.pallas.tpu as pltpu

F32 = jnp.float32
BF16 = jnp.bfloat16

_EPS = 1e-5
_GELU_C = math.sqrt(2.0 / math.pi)
_GELU_A = 0.044715

_ROWS = 8
_TILE = 8

_READ_SLABS = 8
_READ_ROWS = 16
_READ_TAIL = 64
_READ_COLS = 256
_WRITE_SLABS = 8
_WRITE_ROWS = 112

_XG, _W3, _W4, _WQ, _WO, _KV, _KV_TAIL = range(7)
_DK, _DV, _DWQ, _DWO, _DW3, _DW4, _RES = range(7)

_NN = (((1,), (0,)), ((), ()))
_NT = (((1,), (1,)), ((), ()))
_TN = (((0,), (0,)), ((), ()))


def _dot(a, b, dims):
    return lax.dot_general(a.astype(BF16), b.astype(BF16), dims, preferred_element_type=F32)


def _layernorm(x):
    d = x - jnp.mean(x, axis=-1, keepdims=True)
    rstd = 1.0 / jnp.sqrt(jnp.mean(d * d, axis=-1, keepdims=True) + _EPS)
    return d * rstd, rstd


def _layernorm_bwd(dy, y, rstd):
    return rstd * (
        dy - jnp.mean(dy, axis=-1, keepdims=True) - y * jnp.mean(dy * y, axis=-1, keepdims=True)
    )


def _loop(lo, hi, body):
    def step(i, carry):
        body(i)
        return carry

    lax.fori_loop(lo, hi, step, 0)


def _block(i, n):
    return pl.ds(pl.multiple_of(i * n, n), n)


def _matrix(ref):
    return ref[...].reshape(ref.shape[0] * ref.shape[1], ref.shape[2])


def _kernel(
    x_hbm, g_hbm, k_hbm, v_hbm, wq_hbm, wo_hbm, w3_hbm, w4_hbm,
    out_hbm, dx_hbm, dk_hbm, dv_hbm, dwq_hbm, dwo_hbm, dw3_hbm, dw4_hbm,
    xg_buf, pad_buf, res_buf,
    kv_buf, dk_buf, dv_buf, zero_buf,
    wq_buf, wo_buf, w3_buf, w4_buf, dwq_buf, dwo_buf, dw3_buf, dw4_buf,
    q_buf, do_buf, o_buf, dq_buf,
    sems,
):
    batch = x_hbm.shape[0]
    _, slabs, window, dh = kv_buf.shape
    first = k_hbm.shape[1] - window
    kv_heads = slabs // batch
    rep = wq_hbm.shape[2] // (kv_heads * dh)
    groups = dk_hbm.shape[1]
    scale = dh ** -0.5

    def start(src, dst, sem, priority=0):
        pltpu.make_async_copy(src, dst, sems.at[sem]).start(priority=priority)

    def wait_filled(ref, sem):
        pltpu.make_async_copy(ref, ref, sems.at[sem]).wait()

    start(x_hbm, xg_buf.at[0], _XG, priority=0)
    start(g_hbm, xg_buf.at[1], _XG, priority=1)

    def read_weights(wide_hbm, wide_buf, wide_sem, tall_hbm, tall_buf, tall_sem):
        per_row = wide_hbm.shape[2] // _READ_COLS
        steps = tall_hbm.shape[1] // _TILE
        per_step = wide_hbm.shape[1] // _TILE * per_row // steps
        assert steps * per_step == wide_hbm.shape[1] // _TILE * per_row

        def step(i):
            for n in range(per_step):
                r = _block(lax.div(i * per_step + n, per_row), _TILE)
                c = _block(lax.rem(i * per_step + n, per_row), _READ_COLS)
                start(wide_hbm.at[:, r, c], wide_buf.at[:, r, c], wide_sem, priority=0)
            r = _block(i, _TILE)
            start(tall_hbm.at[:, r], tall_buf.at[:, r], tall_sem, priority=1)

        _loop(0, steps, step)

    read_weights(w3_hbm, w3_buf, _W3, w4_hbm, w4_buf, _W4)
    read_weights(wq_hbm, wq_buf, _WQ, wo_hbm, wo_buf, _WO)

    def read_kv(lo, hi, sem):
        def group(n):
            b = pl.ds(n * _READ_SLABS, _READ_SLABS)

            def step(i):
                r = pl.multiple_of(i * _READ_ROWS, _READ_ROWS)
                src, dst = pl.ds(first + r, _READ_ROWS), pl.ds(r, _READ_ROWS)
                start(k_hbm.at[b, src], kv_buf.at[0, b, dst], sem, priority=0)
                start(v_hbm.at[b, src], kv_buf.at[1, b, dst], sem, priority=1)

            _loop(lo // _READ_ROWS, hi // _READ_ROWS, step)

        _loop(0, slabs // _READ_SLABS, group)

    early = window - _READ_TAIL
    assert early % _READ_ROWS == 0 and window % _READ_ROWS == 0 and slabs % _READ_SLABS == 0
    read_kv(0, early, _KV)
    read_kv(early, window, _KV_TAIL)

    zero_buf[...] = jnp.zeros(zero_buf.shape, BF16)
    pad_buf[...] = jnp.zeros(pad_buf.shape, F32)

    for buf, sem in ((xg_buf, _XG), (w3_buf, _W3), (w4_buf, _W4), (wq_buf, _WQ), (wo_buf, _WO)):
        wait_filled(buf, sem)
    wait_filled(kv_buf.at[:, :, pl.ds(0, early)], _KV)

    def sweep(rows, write):
        full, rest = divmod(rows, _WRITE_ROWS)
        _loop(0, full, lambda i: write(pl.multiple_of(i * _WRITE_ROWS, _TILE), _WRITE_ROWS))
        if rest:
            write(full * _WRITE_ROWS, rest)

    def write_zeros(dst, sem, group):
        sweep(first, lambda r, n: start(zero_buf.at[:, pl.ds(0, n)], dst.at[:, group, pl.ds(r, n)], sem))

    write_zeros(dk_hbm, _DK, 0)
    wait_filled(kv_buf.at[:, :, pl.ds(early, _READ_TAIL)], _KV_TAIL)

    pad_buf[0, 0:batch, :] = xg_buf[0].astype(F32)
    pad_buf[1, 0:batch, :] = xg_buf[1].astype(F32)
    x = pad_buf[0]
    g = pad_buf[1]

    xn, rstd1 = _layernorm(x)
    ln2, rstd2 = _layernorm(xn)
    u = _dot(ln2, _matrix(w3_buf), _NN)
    t = jnp.tanh(_GELU_C * (u + _GELU_A * u * u * u))
    a = 0.5 * u * (1.0 + t)
    y = xn + _dot(a, _matrix(w4_buf), _NN)
    sig = jax.nn.sigmoid(y)
    gate = y * sig
    ds = g * gate

    row = lax.broadcasted_iota(jnp.int32, (_ROWS, dh), 0)

    def to_slabs(full, ref):
        for h in range(kv_heads):
            tiles = [full[:, (h * rep + r) * dh:(h * rep + r + 1) * dh] for r in range(rep)]
            for b in range(batch):
                acc = jnp.zeros((_ROWS, dh), F32)
                for r in range(rep):
                    acc = jnp.where(row == r, tiles[r][b:b + 1, :], acc)
                ref[b * kv_heads + h] = acc

    def from_slabs(ref):
        cols = []
        for h in range(kv_heads):
            tiles = [ref[b * kv_heads + h] for b in range(batch)]
            for r in range(rep):
                acc = jnp.zeros((_ROWS, dh), F32)
                for b in range(batch):
                    acc = jnp.where(row == b, tiles[b][r:r + 1, :], acc)
                cols.append(acc)
        return jnp.concatenate(cols, axis=1)

    to_slabs(_dot(xn, _matrix(wq_buf), _NN), q_buf)
    to_slabs(_dot(ds, _matrix(wo_buf), _NT), do_buf)

    def attend(j):
        q, do, k, v = q_buf[j], do_buf[j], kv_buf[0, j], kv_buf[1, j]
        s = _dot(q, k, _NT) * scale
        e = jnp.exp(s - jnp.max(s, axis=-1, keepdims=True))
        p = e / jnp.sum(e, axis=-1, keepdims=True)
        dp = _dot(do, v, _NT)
        dsc = p * (dp - jnp.sum(p * dp, axis=-1, keepdims=True)) * scale
        o_buf[j] = _dot(p, v, _NN)
        dq_buf[j] = _dot(dsc, k, _NN)
        zero = jnp.zeros((_ROWS, dh), F32)
        rhs = jnp.concatenate(
            [jnp.concatenate([do, zero], axis=1), jnp.concatenate([zero, q], axis=1)], axis=0
        )
        dvk = _dot(jnp.concatenate([p, dsc], axis=0), rhs, _TN).astype(BF16)
        dv_buf[lax.div(j, groups), lax.rem(j, groups)] = dvk[:, :dh]
        dk_buf[lax.div(j, groups), lax.rem(j, groups)] = dvk[:, dh:]

    per_sweep = slabs // (2 * groups)

    def step(i):
        @pl.when(i + 1 < groups)
        def _():
            write_zeros(dk_hbm, _DK, i + 1)

        @pl.when(jnp.logical_and(i + 1 >= groups, i + 1 < 2 * groups))
        def _():
            write_zeros(dv_hbm, _DV, i + 1 - groups)

        _loop(i * per_sweep, (i + 1) * per_sweep, attend)

    _loop(0, 2 * groups, step)

    def write_grads(src, dst, sem):
        _loop(0, groups, lambda group: sweep(window, lambda r, n: start(
            src.at[:, group, pl.ds(r, n)], dst.at[:, group, pl.ds(first + r, n)], sem)))

    write_grads(dk_buf, dk_hbm, _DK)
    write_grads(dv_buf, dv_hbm, _DV)

    o = from_slabs(o_buf)
    dq = from_slabs(dq_buf)
    s = _dot(o, _matrix(wo_buf), _NN)
    dy = g * s * sig * (1.0 + y * (1.0 - sig))
    da = _dot(dy, _matrix(w4_buf), _NT)
    du = da * (0.5 * (1.0 + t) + 0.5 * u * (1.0 - t * t) * _GELU_C * (1.0 + 3.0 * _GELU_A * u * u))
    dxn = (
        dy
        + _layernorm_bwd(_dot(du, _matrix(w3_buf), _NT), ln2, rstd2)
        + _dot(dq, _matrix(wq_buf), _NT)
    )
    res_buf[0] = (x + s * gate)[0:batch].astype(BF16)
    res_buf[1] = (g + _layernorm_bwd(dxn, xn, rstd1))[0:batch].astype(BF16)
    for ref, lhs, rhs in ((dwq_buf, xn, dq), (dwo_buf, o, ds), (dw3_buf, ln2, du), (dw4_buf, a, dy)):
        ref[...] = _dot(lhs, rhs, _TN).astype(BF16).reshape(ref.shape)

    results = [
        pltpu.make_async_copy(res_buf.at[n], dst, sems.at[_RES])
        for n, dst in enumerate((out_hbm, dx_hbm))
    ]
    for copy in results:
        copy.start()

    def write_part(src, dst, sem, *index):
        index = (slice(None),) + index
        start(src.at[index], dst.at[index], sem)

    tall = 4 * _TILE

    def write_weights(i):
        cols = _block(lax.rem(i, 2), dwq_buf.shape[2] // 2)
        write_part(dwq_buf, dwq_hbm, _DWQ, _block(lax.div(i, 2), _TILE), cols)

        @pl.when(i < dw3_buf.shape[1] // _TILE)
        def _():
            write_part(dw3_buf, dw3_hbm, _DW3, _block(i, _TILE))

        write_part(dwo_buf, dwo_hbm, _DWO, _block(i, tall))

        @pl.when(i < dw4_buf.shape[1] // tall)
        def _():
            write_part(dw4_buf, dw4_hbm, _DW4, _block(i, tall))

    steps = dwo_buf.shape[1] // tall
    assert steps == 2 * dwq_buf.shape[1] // _TILE
    assert dw3_buf.shape[1] // _TILE <= steps and dw4_buf.shape[1] // tall <= steps
    _loop(0, steps, write_weights)

    for copy in results:
        copy.wait()
    for ref, sem in (
        (dk_hbm, _DK), (dv_hbm, _DV), (dw4_hbm, _DW4), (dw3_hbm, _DW3), (dwq_hbm, _DWQ), (dwo_hbm, _DWO),
    ):
        wait_filled(ref, sem)


@jax.jit
def pallas_recurrent_scan__sliding_block_cached__mixer_s_mlp__decode_kernel(
    A_x: jax.Array,
    A_k_cache: jax.Array,
    A_v_cache: jax.Array,
    A_wq: jax.Array,
    A_wo: jax.Array,
    B_x: jax.Array,
    B_w1: jax.Array,
    B_w2: jax.Array,
    B_w3: jax.Array,
    B_w4: jax.Array,
    grad_out: jax.Array,
):
    del B_x, B_w1, B_w2
    batch, seq, dim = A_x.shape
    _, kv_heads, keys, dh = A_k_cache.shape
    assert seq == 1 and batch <= _ROWS
    window = min(4096, max(256, keys // 4))
    slabs = batch * kv_heads
    groups = slabs // _WRITE_SLABS

    def split(w, n):
        return (n, w.shape[0] // n, w.shape[1])

    weights = (A_wq, A_wo, B_w3, B_w4)
    read_shapes = [split(w, 4) for w in weights]
    write_shapes = [split(w, n) for w, n in zip(weights, (2, 2, 1, 1))]

    hbm = pl.BlockSpec(memory_space=pltpu.HBM)
    out, dx, dk, dv, *dws = pl.pallas_call(
        _kernel,
        in_specs=[hbm] * 8,
        out_specs=[hbm] * 8,
        out_shape=[
            jax.ShapeDtypeStruct(shape, BF16)
            for shape in [(batch, dim)] * 2 + [(_WRITE_SLABS, groups, keys, dh)] * 2 + write_shapes
        ],
        scratch_shapes=[
            pltpu.VMEM((2, batch, dim), BF16),
            pltpu.VMEM((2, _ROWS, dim), F32),
            pltpu.VMEM((2, batch, dim), BF16),
            pltpu.VMEM((2, slabs, window, dh), BF16),
            *[pltpu.VMEM((_WRITE_SLABS, groups, window, dh), BF16)] * 2,
            pltpu.VMEM((_WRITE_SLABS, _WRITE_ROWS, dh), BF16),
            *[pltpu.VMEM(shape, BF16) for shape in read_shapes + write_shapes],
            *[pltpu.VMEM((slabs, _ROWS, dh), F32)] * 4,
            pltpu.SemaphoreType.DMA((7,)),
        ],
        compiler_params=pltpu.CompilerParams(vmem_limit_bytes=100 << 20),
        name="window_attention_mixer_fwd_bwd",
    )(
        A_x.reshape(batch, dim),
        grad_out.reshape(batch, dim),
        A_k_cache.reshape(slabs, keys, dh),
        A_v_cache.reshape(slabs, keys, dh),
        *[w.reshape(shape) for w, shape in zip(weights, read_shapes)],
    )
    return (
        out.reshape(A_x.shape),
        dx.reshape(A_x.shape),
        dk.reshape(A_k_cache.shape),
        dv.reshape(A_v_cache.shape),
        *[dw.reshape(w.shape) for dw, w in zip(dws, weights)],
    )
```
